```python
import os as _os
_os.environ.setdefault("JAX_PLATFORMS", "cpu")
import jax
import jax.numpy as jnp

def _softmax(x, axis=-1):
    return jax.nn.softmax(x, axis=axis)
def _gelu(x):
    return jax.nn.gelu(x, approximate=True)
def _silu(x):
    return jax.nn.silu(x)
def _sigmoid(x):
    return jax.nn.sigmoid(x)
def _layernorm(x, axis=-1, eps=1e-5):
    m = jnp.mean(x, axis=axis, keepdims=True)
    v = jnp.var(x, axis=axis, keepdims=True)
    return (x - m) / jnp.sqrt(v + eps)
def _scatter_add(tgt, idx, src, axis=0):
    return tgt.at[idx].add(src)
def _segment_sum(src, seg, n):
    return jax.ops.segment_sum(src, seg, n)
class _Rng:
    def __init__(self, key):
        self._k = key
    def _next(self):
        self._k, sub = jax.random.split(self._k)
        return sub
    def normal(self, shape):
        return jax.random.normal(self._next(), shape, dtype=jnp.bfloat16)
    def randint(self, lo, hi, shape):
        return jax.random.randint(self._next(), shape, lo, hi, dtype=jnp.int32)
    def uniform(self, shape, lo=0.0, hi=1.0):
        return jax.random.uniform(self._next(), shape, jnp.bfloat16, lo, hi)
    def permutation(self, n):
        return jax.random.permutation(self._next(), n)


kernel_name = 'sequential_preLN__mha_block__swiglu_ffn__prompt'

def setup_inputs():
    _rng = _Rng(jax.random.key(int.from_bytes(__import__("os").urandom(4), "little")))
    _w = (lambda a: (lambda t: t.astype(jnp.bfloat16) if jnp.issubdtype(t.dtype, jnp.floating) else t)(jnp.asarray(a)))
    def _A_setup():
        B, S, D, H = 1, 2048, 640, 32
        return {
            "x": _w((lambda *s: _rng.normal(s) * 0.05)(B, S, D)),
            "wqkv": _w((lambda *s: _rng.normal(s) * 0.05)(D, 3 * D)),
            "wo": _w((lambda *s: _rng.normal(s) * 0.05)(D, D)),
        }
    _A_in = _A_setup()

    def _B_setup():
        B, S, D, F = 1, 2048, 640, 1728
        return {
            "x": _w((lambda *s: _rng.normal(s) * 0.05)(B, S, D)),
            "w_gate": _w((lambda *s: _rng.normal(s) * 0.05)(D, F)),
            "w_up": _w((lambda *s: _rng.normal(s) * 0.05)(D, F)),
            "w_down": _w((lambda *s: _rng.normal(s) * 0.05)(F, D)),
        }
    _B_in = _B_setup()

    return {
        "A_x": _A_in["x"],
        "A_wqkv": _A_in["wqkv"],
        "A_wo": _A_in["wo"],
        "B_x": _B_in["x"],
        "B_w_gate": _B_in["w_gate"],
        "B_w_up": _B_in["w_up"],
        "B_w_down": _B_in["w_down"],
    }

def reference(A_x, A_wqkv, A_wo, B_x, B_w_gate, B_w_up, B_w_down):
    def _A_ref(x, wqkv, wo):
        B, S, D = x.shape
        H = 32
        Dh = D // H
        qkv = (lambda x, *d: x.transpose(*d))((x @ wqkv).reshape(B, S, 3, H, Dh), 2, 0, 3, 1, 4)
        q, k, v = qkv[0], qkv[1], qkv[2]
        scores = jnp.einsum("bhqd,bhkd->bhqk", q, k) * (Dh ** -0.5)
        p = _softmax(scores, axis=-1)
        o = jnp.einsum("bhqk,bhkd->bhqd", p, v)
        return (lambda x, *d: x.transpose(*d))(o, 0, 2, 1, 3).reshape(B, S, D) @ wo

    def _B_ref(x, w_gate, w_up, w_down):
        g = _silu(x @ w_gate)
        u = x @ w_up
        return (g * u) @ w_down

    x = A_x
    h = x + _A_ref(_layernorm(x, axis=-1), A_wqkv, A_wo)
    h2 = h + _B_ref(_layernorm(h, axis=-1), B_w_gate, B_w_up, B_w_down)
    return h2
```

```python
import jax
import jax.numpy as jnp
from jax import lax
import jax.experimental.pallas as pl
import jax.experimental.pallas.tpu as pltpu

S, D, H, DH, F = 2048, 640, 32, 20, 1728
BM = 512
CK = 128
CQ = 512
EPS = 1e-5
QSCALE = (DH ** -0.5) * 1.4426950408889634
NT = (((1,), (1,)), ((), ()))
TN = (((0,), (0,)), ((), ()))
f32, bf16 = jnp.float32, jnp.bfloat16


FM = F // 128 * 128
FT = F - FM
LC = 64
ET = 128
OB = 128
u32 = jnp.uint32
def _pk(v):
    return pltpu.bitcast(v.astype(bf16), u32)
def _unpk(v):
    return pltpu.bitcast(v, bf16)
def _ln(v):
    mu = jnp.mean(v, axis=-1, keepdims=True)
    d = v - mu
    var = jnp.mean(d * d, axis=-1, keepdims=True)
    return d * lax.rsqrt(var + EPS)


def _kernel(x_hbm, wqkv_hbm, wo_hbm, wg_hbm, wu_hbm, wd_hbm, out_hbm,
            x_v, wqkv_v, wo_v, wgu_v, wd_v, xn_s, h_s, wqvT, qT_s, k_s, vT_s, oT_s,
            qm_s, s0, s1, m0, m1, out_v, sems, osems):
    NB = S // BM
    x_cp = [pltpu.make_async_copy(x_hbm.at[pl.ds(b * BM, BM)], x_v.at[pl.ds(b * BM, BM)], sems.at[b]) for b in range(NB)]
    qkv_cp = [pltpu.make_async_copy(wqkv_hbm.at[:, pl.ds(i * D, D)], wqkv_v.at[:, pl.ds(i * D, D)], sems.at[NB + i])
              for i in range(3)]
    w_cp = [pltpu.make_async_copy(src, dst, sems.at[NB + 3 + i]) for i, (src, dst) in enumerate([
        (wo_hbm, wo_v),
        (wg_hbm.at[pl.ds(0, FM)], wgu_v.at[pl.ds(0, FM)]),
        (wu_hbm.at[pl.ds(0, FM)], wgu_v.at[pl.ds(FM, FM)]),
        (wg_hbm.at[pl.ds(FM, FT)], wgu_v.at[pl.ds(2 * FM, FT)]),
        (wu_hbm.at[pl.ds(FM, FT)], wgu_v.at[pl.ds(2 * FM + FT, FT)]),
        (wd_hbm, wd_v.at[pl.ds(0, F)])])]
    x_cp[0].start()
    qkv_cp[1].start()

    def ln1(b):
        for r in range(b * BM, (b + 1) * BM, LC):
            xn_s[r:r + LC, :] = _ln(x_v[r:r + LC, :].astype(f32)).astype(bf16)

    def ln2(r0):
        for r in range(0, ET, LC):
            rows = pl.ds(r0 + r, LC)
            xn_s[rows, :] = _ln(h_s[rows, :]).astype(bf16)

    def k_proj(r0, n):
        k = jnp.dot(xn_s[pl.ds(r0, n), :], wqkv_v[:, D:2 * D], preferred_element_type=f32)
        kg = [k[:, g * 128:(g + 1) * 128] for g in range(5)]
        prow = slice(r0 // 2, (r0 + n) // 2)
        hi = lax.broadcasted_iota(jnp.int32, (n, 128), 1) >= 64
        for g in range(5):
            k_s[g, prow, :] = _pk(kg[g])
        for g in range(4):
            k_s[5 + g, prow, :] = _pk(jnp.where(hi, kg[g], kg[g + 1]))

    x_cp[0].wait()
    for c in x_cp[1:]:
        c.start()
    ln1(0)
    wd_v[F:FM + 2 * FT, :] = jnp.zeros((FT, D), bf16)
    qkv_cp[1].wait()
    lane = lax.broadcasted_iota(jnp.int32, (BM, 128), 1)
    k_proj(0, 384)
    for c in x_cp[1:]:
        c.wait()
    qkv_cp[0].start()
    qkv_cp[2].start()
    k_proj(384, 128)
    for b in range(1, NB):
        ln1(b)
    for r0 in range(BM, S - 256, 256):
        k_proj(r0, 256)
    qkv_cp[0].wait()
    qkv_cp[2].wait()
    for c in w_cp:
        c.start()
    k_proj(S - 256, 256)
    wqvT[0:D, :] = wqkv_v[:, 0:D].T
    wqvT[D:2 * D, :] = wqkv_v[:, 2 * D:3 * D].T
    for b in range(NB):
        rows = slice(b * BM, (b + 1) * BM)
        qv = lax.dot_general(wqvT[...], xn_s[rows, :], NT, preferred_element_type=f32)
        qT_s[:, rows] = _pk(qv[0:D] * QSCALE)
        vT_s[:, rows] = qv[D:2 * D]

    def put_q(h):
        start = h * DH
        g = start // 128
        off = start % 128
        strad = (off > 128 - DH).astype(jnp.int32) if not isinstance(h, int) else int(off > 128 - DH)
        top = qT_s[pl.ds(pl.multiple_of((g + strad) * 64, 64), 32), :]
        bot = qT_s[pl.ds(pl.multiple_of(g * 64 + 32, 32), 32), :]
        r = 2 * lax.broadcasted_iota(jnp.int32, (32, S), 0)
        top = jnp.where(((r - off) & 127) < DH, top, jnp.zeros_like(top))
        bot = jnp.where(((r + 64 - off) & 127) < DH, bot, jnp.zeros_like(bot))
        qm_s[0:32, :] = top
        qm_s[32:64, :] = bot
        return g + 5 * strad

    def qk_chunk(kgi, c, js, s_nxt):
        s = jnp.dot(_unpk(k_s[kgi, c * CK // 2:(c + 1) * CK // 2, :]), _unpk(qm_s[:, js]), preferred_element_type=f32)
        s_nxt[c * CK:(c + 1) * CK, js] = s
        return jnp.max(s.reshape(CK // 8, 8, CQ), axis=0)

    def v_win(h, odd, c):
        w0 = pl.multiple_of(h * DH - 4 * odd, 8)
        v = vT_s[pl.ds(w0, 24), c * CK:(c + 1) * CK]
        r = lax.broadcasted_iota(jnp.int32, (8, CK), 0)
        if odd:
            return jnp.concatenate([jnp.where(r < 4, 1.0, v[0:8]), v[8:24]], axis=0)
        return jnp.concatenate([v[0:16], jnp.where(r >= 4, 1.0, v[16:24])], axis=0)

    def pv_chunk(h, odd, c, js, s_cur, m):
        sc = s_cur[c * CK:(c + 1) * CK, js].reshape(CK // 8, 8, -1)
        p = jnp.exp2(sc - m[None]).reshape(CK, -1)
        return jnp.dot(v_win(h, odd, c), p, preferred_element_type=f32)

    def put_o(h, odd, js, acc):
        w0 = pl.multiple_of(h * DH - 4 * odd, 8)
        l = acc[0:1] if odd else acc[23:24]
        o = acc * (1.0 / l)
        if odd:
            r = lax.broadcasted_iota(jnp.int32, (8, acc.shape[1]), 0)
            oT_s[pl.ds(w0, 8), js] = jnp.where(r >= 4, o[0:8], oT_s[pl.ds(w0, 8), js])
            oT_s[pl.ds(w0 + 8, 16), js] = o[8:24]
        else:
            oT_s[pl.ds(w0, 24), js] = o

    def stage(h, odd, s_cur, m_cur, s_nxt, m_nxt):
        kgi = put_q(h + 1)
        for j in range(S // CQ):
            js = slice(j * CQ, (j + 1) * CQ)
            m = m_cur[:, js]
            mx = acc = None
            for c in range(S // CK):
                cm = qk_chunk(kgi, c, js, s_nxt)
                mx = cm if mx is None else jnp.maximum(mx, cm)
                o = pv_chunk(h, odd, c, js, s_cur, m)
                acc = o if acc is None else acc + o
            m_nxt[:, js] = jnp.broadcast_to(jnp.max(mx, axis=0, keepdims=True), (8, CQ))
            put_o(h, odd, js, acc)

    kgi = put_q(0)
    for j in range(S // CQ):
        js = slice(j * CQ, (j + 1) * CQ)
        mx = None
        for c in range(S // CK):
            cm = qk_chunk(kgi, c, js, s0)
            mx = cm if mx is None else jnp.maximum(mx, cm)
        m0[:, js] = jnp.broadcast_to(jnp.max(mx, axis=0, keepdims=True), (8, CQ))

    def body(h, carry):
        @pl.when(h % 2 == 0)
        def _():
            stage(h, 0, s0, m0, s1, m1)

        @pl.when(h % 2 == 1)
        def _():
            stage(h, 1, s1, m1, s0, m0)
        return carry

    lax.fori_loop(0, H - 1, body, 0)
    for c in w_cp:
        c.wait()

    for j in range(S // ET + 1):
        if j < S // ET:
            js = slice(j * ET, (j + 1) * ET)
            m = m1[:, js]
            for c in range(S // CK):
                o = pv_chunk(H - 1, 1, c, js, s1, m)
                acc = o if c == 0 else acc + o
            put_o(H - 1, 1, js, acc)
        if j > 0:
            js = slice((j - 1) * ET, j * ET)
            a = lax.dot_general(oT_s[:, js].astype(bf16), wo_v[...], TN, preferred_element_type=f32)
            h_s[js, :] = x_v[js, :].astype(f32) + a
            ln2(js.start)

    def out_cp(b):
        r0 = pl.multiple_of(b * OB, OB)
        return pltpu.make_async_copy(out_v.at[pl.ds(r0, OB)], out_hbm.at[pl.ds(r0, OB)], osems.at[b])

    def ffn(b, carry):
        rows = pl.ds(pl.multiple_of(b * BM, BM), BM)
        hn = xn_s[rows, :]
        t = lax.dot_general(hn, wgu_v[2 * FM:2 * FM + 2 * FT, :], NT, preferred_element_type=f32)
        at = jnp.where(lane < FT, t * jax.nn.sigmoid(t) * pltpu.roll(t, FT, 1), 0.0).astype(bf16)
        g = lax.dot_general(hn, wgu_v[0:FM, :], NT, preferred_element_type=f32)
        u = lax.dot_general(hn, wgu_v[FM:2 * FM, :], NT, preferred_element_type=f32)
        act = jnp.concatenate([(g * jax.nn.sigmoid(g) * u).astype(bf16), at], axis=1)
        for i in range(BM // OB):
            y = jnp.dot(act[i * OB:(i + 1) * OB], wd_v[...], preferred_element_type=f32)
            orow = pl.ds(pl.multiple_of(b * BM + i * OB, OB), OB)
            out_v[orow, :] = (h_s[orow, :] + y).astype(bf16)
            out_cp(b * (BM // OB) + i).start()
        return carry

    lax.fori_loop(0, NB, ffn, 0)
    for b in range(S // OB):
        out_cp(b).wait()


@jax.jit
def pallas_sequential_preLN__mha_block__swiglu_ffn__prompt_kernel(A_x, A_wqkv, A_wo, B_x, B_w_gate, B_w_up, B_w_down):
    del B_x
    any_spec = pl.BlockSpec(memory_space=pl.ANY)
    out = pl.pallas_call(
        _kernel,
        out_shape=jax.ShapeDtypeStruct((S, D), bf16),
        in_specs=[any_spec] * 6,
        out_specs=any_spec,
        scratch_shapes=[
            pltpu.VMEM((S, D), bf16), pltpu.VMEM((D, 3 * D), bf16), pltpu.VMEM((D, D), bf16),
            pltpu.VMEM((2 * F, D), bf16), pltpu.VMEM((FM + 2 * FT, D), bf16), pltpu.VMEM((S, D), bf16), pltpu.VMEM((S, D), f32),
            pltpu.VMEM((2 * D, D), bf16), pltpu.VMEM((D // 2, S), u32), pltpu.VMEM((9, S // 2, 128), u32),
            pltpu.VMEM((D, S), f32), pltpu.VMEM((D, S), f32), pltpu.VMEM((64, S), u32),
            pltpu.VMEM((S, S), f32), pltpu.VMEM((S, S), f32), pltpu.VMEM((8, S), f32), pltpu.VMEM((8, S), f32),
            pltpu.VMEM((S, D), bf16),
            pltpu.SemaphoreType.DMA((S // BM + 9,)), pltpu.SemaphoreType.DMA((S // OB,)),
        ],
        compiler_params=pltpu.CompilerParams(vmem_limit_bytes=110 * 1024 * 1024),
    )(A_x.reshape(S, D), A_wqkv, A_wo, B_w_gate.T, B_w_up.T, B_w_down)
    return out.reshape(1, S, D)
```
